```python
import os as _os
_os.environ.setdefault("JAX_PLATFORMS", "cpu")
import jax
import jax.numpy as jnp

def _softmax(x, axis=-1):
    return jax.nn.softmax(x, axis=axis)
def _gelu(x):
    return jax.nn.gelu(x, approximate=True)
def _silu(x):
    return jax.nn.silu(x)
def _sigmoid(x):
    return jax.nn.sigmoid(x)
def _layernorm(x, axis=-1, eps=1e-5):
    m = jnp.mean(x, axis=axis, keepdims=True)
    v = jnp.var(x, axis=axis, keepdims=True)
    return (x - m) / jnp.sqrt(v + eps)
def _scatter_add(tgt, idx, src, axis=0):
    return tgt.at[idx].add(src)
def _segment_sum(src, seg, n):
    return jax.ops.segment_sum(src, seg, n)
class _Rng:
    def __init__(self, key):
        self._k = key
    def _next(self):
        self._k, sub = jax.random.split(self._k)
        return sub
    def normal(self, shape):
        return jax.random.normal(self._next(), shape, dtype=jnp.bfloat16)
    def randint(self, lo, hi, shape):
        return jax.random.randint(self._next(), shape, lo, hi, dtype=jnp.int32)
    def uniform(self, shape, lo=0.0, hi=1.0):
        return jax.random.uniform(self._next(), shape, jnp.bfloat16, lo, hi)
    def permutation(self, n):
        return jax.random.permutation(self._next(), n)


kernel_name = 'parallel_sum__ssm_conv_s4__mixer_channel_mlp__prompt'

def setup_inputs():
    _rng = _Rng(jax.random.key(int.from_bytes(__import__("os").urandom(4), "little")))
    _w = (lambda a: (lambda t: t.astype(jnp.bfloat16) if jnp.issubdtype(t.dtype, jnp.floating) else t)(jnp.asarray(a)))
    def _A_setup():
        B, L, D, N = 1, 2048, 512, 128
        A_re = -jnp.exp((lambda *s: _rng.normal(s) * 0.1)(D, N))
        A_im = jnp.pi * (lambda *s: _rng.normal(s) * 0.1)(D, N)
        B_re = (lambda *s: _rng.normal(s) * 0.1)(D, N)
        B_im = (lambda *s: _rng.normal(s) * 0.1)(D, N)
        C_re = (lambda *s: _rng.normal(s) * 0.1)(D, N)
        C_im = (lambda *s: _rng.normal(s) * 0.1)(D, N)
        log_dt = (lambda *s: _rng.normal(s) * 0.1)(D) * 0.5 - 4.0
        Dskip = (lambda *s: _rng.normal(s) * 0.05)(D)
        return {
            "u": _w((lambda *s: _rng.normal(s) * 0.05)(B, L, D)),
            "A_re": _w(A_re),
            "A_im": _w(A_im),
            "B_re": _w(B_re),
            "B_im": _w(B_im),
            "C_re": _w(C_re),
            "C_im": _w(C_im),
            "log_dt": _w(log_dt),
            "Dskip": _w(Dskip),
        }
    _A_in = _A_setup()

    def _B_setup():
        B, S, D, F = 1, 2048, 512, 1792
        return {
            "x": _w((lambda *s: _rng.normal(s) * 0.05)(B, S, D)),
            "w1": _w((lambda *s: _rng.normal(s) * 0.2)(D, F) * (D ** -0.5)),
            "b1": _w((lambda *s: _rng.normal(s) * 0.2)(F)),
            "w2": _w((lambda *s: _rng.normal(s) * 0.2)(F, D) * (F ** -0.5)),
            "b2": _w((lambda *s: _rng.normal(s) * 0.05)(D)),
        }
    _B_in = _B_setup()

    return {
        "A_u": _A_in["u"],
        "A_A_re": _A_in["A_re"],
        "A_A_im": _A_in["A_im"],
        "A_B_re": _A_in["B_re"],
        "A_B_im": _A_in["B_im"],
        "A_C_re": _A_in["C_re"],
        "A_C_im": _A_in["C_im"],
        "A_log_dt": _A_in["log_dt"],
        "A_Dskip": _A_in["Dskip"],
        "B_x": _B_in["x"],
        "B_w1": _B_in["w1"],
        "B_b1": _B_in["b1"],
        "B_w2": _B_in["w2"],
        "B_b2": _B_in["b2"],
    }

def reference(A_u, A_A_re, A_A_im, A_B_re, A_B_im, A_C_re, A_C_im, A_log_dt, A_Dskip, B_x, B_w1, B_b1, B_w2, B_b2):
    def _A_ref(u, A_re, A_im, B_re, B_im, C_re, C_im, log_dt, Dskip):
        Bsz, L, D = u.shape
        dt = jnp.exp(log_dt)[:, None]
        A = A_re + 1j * A_im
        Bc = B_re + 1j * B_im
        Cc = C_re + 1j * C_im
        logdA = dt * A
        dB = dt * Bc
        l = (lambda x, dt: x.astype(dt))(jnp.arange(L), A_re.dtype)
        P = jnp.exp(logdA[:, :, None] * l[None, None, :])
        K = jnp.einsum("dn,dnl,dn->dl", Cc, P, dB).real
        L2 = 2 * L
        Kp = jnp.pad(K, ((0, 0), (0, L)))
        up = (lambda x, *d: x.transpose(*d))(u, 0, 2, 1)
        up = jnp.pad(up, ((0, 0), (0, 0), (0, L)))
        Kf = (lambda x, axes=(-2,-1): jnp.fft.rfft2(x.astype(jnp.float32), axes=axes))(Kp[:, None, :], axes=(-2, -1))
        Uf = (lambda x, axes=(-2,-1): jnp.fft.rfft2(x.astype(jnp.float32), axes=axes))(up[:, :, None, :], axes=(-2, -1))
        Yf = Uf * Kf[None, :, :, :]
        y = (lambda x, s, axes=(-2,-1): jnp.fft.irfft2(x, s=s, axes=axes).astype(jnp.bfloat16))(Yf, (1, L2), axes=(-2, -1))[:, :, 0, :L]
        y = (lambda x, *d: x.transpose(*d))(y, 0, 2, 1) + u * Dskip[None, None, :]
        return y

    def _B_ref(x, w1, b1, w2, b2):
        y = _layernorm(x, axis=-1)
        h = _gelu(jnp.einsum("bsd,df->bsf", y, w1) + b1)
        return jnp.einsum("bsf,fd->bsd", h, w2) + b2

    x = A_u
    xn = _layernorm(x, axis=-1)
    return x + _A_ref(xn, A_A_re, A_A_im, A_B_re, A_B_im, A_C_re, A_C_im, A_log_dt, A_Dskip) + _B_ref(xn, B_w1, B_b1, B_w2, B_b2)
```

```python
import numpy as np
import jax
import jax.numpy as jnp
import jax.experimental.pallas as pl
import jax.experimental.pallas.tpu as pltpu

L, D, N, FF = 2048, 512, 128, 1792
B = 128
NB = L // B
NF = 2 * B
EPS = 1e-5

NQ = 81
FROWS = NQ * 8


def _row_lag(row):
    if row < 256:
        return row
    if row < 384:
        return 256 + 2 * (row - 256)
    if row < 512:
        return 512 + 4 * (row - 384)
    return 1024 + 8 * (row - 512)


def _q_level(q):
    return 0 if q < 32 else (1 if q < 48 else (2 if q < 64 else 3))


def _block_rows(d):
    if d < 2:
        return d * B, B
    if d < 4:
        return 256 + (d - 2) * 64, 72
    if d < 8:
        return 384 + (d - 4) * 32, 40
    return 512 + (d - 8) * 16, 24


def _block_new_qs(d):
    def last_q(dd):
        r0, cnt = _block_rows(dd)
        return (r0 + cnt - 1) // 8
    lo = 0 if d == 0 else last_q(d - 1) + 1
    return list(range(lo, last_q(d) + 1))


def _split_bf16(a):
    hi = np.asarray(a, np.float64).astype(jnp.bfloat16)
    lo = (np.asarray(a, np.float64) - hi.astype(np.float64)).astype(jnp.bfloat16)
    return hi, lo


def _make_constants():
    k = np.arange(B)
    l = np.arange(B)
    theta = np.pi * (2 * k + 1) / (2 * B)
    ang = np.outer(theta, l)
    fwd = np.concatenate([np.cos(ang), -np.sin(ang)], 0)
    inv = np.concatenate([np.cos(ang.T), -np.sin(ang.T)], 1) / B
    lag_bf16 = np.arange(L).astype(jnp.bfloat16).astype(np.float64)
    frs = []
    for d in (2, 4, 8):
        r0, cnt = _block_rows(d)
        lags = np.array([_row_lag(r0 + j) for j in range(cnt)], np.float64)
        rep = (lag_bf16[d * B:(d + 1) * B][:, None] == lags[None, :]).astype(np.float64)
        frs.append(fwd @ rep)
    consts = []
    for m in [fwd, inv] + frs:
        consts.extend(_split_bf16(m))
    return consts


def _layernorm(x):
    m = jnp.mean(x, axis=-1, keepdims=True)
    xc = x - m
    v = jnp.mean(xc * xc, axis=-1, keepdims=True)
    return xc * jax.lax.rsqrt(v + EPS)


def _dot(a, b):
    return jnp.dot(a, b, preferred_element_type=jnp.float32)


def _dot3(a_hi, a_lo, b):
    b_hi = b.astype(jnp.bfloat16)
    b_lo = (b - b_hi.astype(jnp.float32)).astype(jnp.bfloat16)
    return _dot(a_hi, b_hi) + (_dot(a_hi, b_lo) + _dot(a_lo, b_hi))


def _cmul(ar, ai, br, bi):
    return ar * br - ai * bi, ar * bi + ai * br


def _kernel(x_ref, are_ref, aim_ref, bre_ref, bim_ref, cre_ref, cim_ref, logdt_ref, dskip_ref,
            w1_ref, b1_ref, w2_ref, b2_ref,
            fhi_ref, flo_ref, ihi_ref, ilo_ref,
            r2hi_ref, r2lo_ref, r4hi_ref, r4lo_ref, r8hi_ref, r8lo_ref,
            o_ref,
            uh_scr, kp_scr, khp_scr, f_scr, pw_re, pw_im, w_re, w_im, g_re, g_im, gc_re, gc_im):
    c = pl.program_id(0)
    f32 = jnp.float32

    @pl.when(c == 0)
    def _setup():
        dt = jnp.exp(logdt_ref[...].astype(f32)).astype(jnp.bfloat16).astype(f32)
        tr = lambda r: r[...].astype(f32).T
        a_r = tr(are_ref) * dt
        a_i = tr(aim_ref) * dt
        db_r = tr(bre_ref) * dt
        db_i = tr(bim_ref) * dt
        c_r = tr(cre_ref)
        c_i = tr(cim_ref)
        cb_r, cb_i = _cmul(c_r, c_i, db_r, db_i)
        gc_re[...] = cb_r
        gc_im[...] = cb_i
        for i in range(7):
            if i % 3 == 0:
                mag = jnp.exp(a_r * float(2 ** i))
                ph = a_i * float(2 ** i)
                er, ei = mag * jnp.cos(ph), mag * jnp.sin(ph)
            else:
                er, ei = er * er - ei * ei, 2.0 * er * ei
            pw_re[i] = er
            pw_im[i] = ei

        sub = jax.lax.broadcasted_iota(jnp.int32, (8, D), 0)
        bits = [(sub & (1 << b)) != 0 for b in range(3)]

        def wbody(n, carry):
            for j in range(4):
                xr = jnp.ones((8, D), f32)
                xi = jnp.zeros((8, D), f32)
                for b in range(3):
                    er_ = pw_re[j + b, pl.ds(n, 1), :]
                    ei_ = pw_im[j + b, pl.ds(n, 1), :]
                    yr = jnp.where(bits[b], er_, 1.0)
                    yi = jnp.where(bits[b], ei_, 0.0)
                    if b == 0:
                        xr, xi = yr, yi
                    else:
                        xr, xi = _cmul(xr, xi, yr, yi)
                w_re[j, n] = xr
                w_im[j, n] = xi
            return carry
        jax.lax.fori_loop(0, N, wbody, 0)
        khp_scr[...] = jnp.zeros_like(khp_scr)

    x = x_ref[...].astype(f32)
    xn_b = _layernorm(x).astype(jnp.bfloat16)
    xn = xn_b.astype(f32)
    uh_scr[c] = _dot(fhi_ref[...], xn_b) + _dot(flo_ref[...], xn_b)

    def kblock(d):
        qs = _block_new_qs(d)
        gr = gc_re[...]
        gi = gc_im[...]
        for i, q in enumerate(qs):
            g_re[i] = gr
            g_im[i] = gi
            lv = _q_level(q)
            gr, gi = _cmul(gr, gi, pw_re[3 + lv], pw_im[3 + lv])
        gc_re[...] = gr
        gc_im[...] = gi
        groups = []
        for i, q in enumerate(qs):
            if groups and _q_level(groups[-1][0][1]) == _q_level(q) and len(groups[-1]) < 8:
                groups[-1].append((i, q))
            else:
                groups.append([(i, q)])
        for grp in groups:
            lv = _q_level(grp[0][1])

            def body(n, accs, grp=grp, lv=lv):
                t_r = w_re[lv, n]
                t_i = w_im[lv, n]
                out = []
                for (i, q), acc in zip(grp, accs):
                    g_r = g_re[i, pl.ds(n, 1), :]
                    g_i = g_im[i, pl.ds(n, 1), :]
                    out.append(acc + (g_r * t_r - g_i * t_i))
                return tuple(out)
            accs = jax.lax.fori_loop(0, N, body, tuple(jnp.zeros((8, D), f32) for _ in grp))
            for (i, q), acc in zip(grp, accs):
                if q == NQ - 1:
                    sub = jax.lax.broadcasted_iota(jnp.int32, (8, D), 0)
                    acc = jnp.where(sub < 1, acc, 0.0)
                f_scr[q * 8:(q + 1) * 8, :] = acc
        r0, cnt = _block_rows(d)
        fb = f_scr[r0:r0 + cnt, :]
        if d < 2:
            m_hi, m_lo = fhi_ref[...], flo_ref[...]
        elif d < 4:
            m_hi, m_lo = r2hi_ref[...], r2lo_ref[...]
        elif d < 8:
            m_hi, m_lo = r4hi_ref[...], r4lo_ref[...]
        else:
            m_hi, m_lo = r8hi_ref[...], r8lo_ref[...]
        kh = _dot3(m_hi, m_lo, fb)
        sgn = jnp.where((jax.lax.broadcasted_iota(jnp.int32, (B, D), 0) & 1) == 0, 1.0, -1.0)
        prev = khp_scr[...]
        kp_scr[d, :B, :] = kh[:B] - sgn * prev[B:]
        kp_scr[d, B:, :] = kh[B:] + sgn * prev[:B]
        khp_scr[...] = kh

    for d in range(NB):
        pl.when(c == d)(lambda d=d: kblock(d))

    RC = 16
    zs = []
    for rc in range(B // RC):
        rows_r = pl.ds(rc * RC, RC)
        rows_i = pl.ds(B + rc * RC, RC)

        def zbody(dl, carry, rows_r=rows_r, rows_i=rows_i):
            zr, zi = carry
            kr = kp_scr[dl, rows_r, :]
            ki = kp_scr[dl, rows_i, :]
            ur = uh_scr[c - dl, rows_r, :]
            ui = uh_scr[c - dl, rows_i, :]
            return zr + (kr * ur - ki * ui), zi + (kr * ui + ki * ur)
        zr, zi = jax.lax.fori_loop(0, c + 1, zbody,
                                   (jnp.zeros((RC, D), f32), jnp.zeros((RC, D), f32)))
        zs.append((zr, zi))
    z = jnp.concatenate([zz[0] for zz in zs] + [zz[1] for zz in zs], axis=0)
    y = _dot3(ihi_ref[...], ilo_ref[...], z)

    y2 = _layernorm(xn).astype(jnp.bfloat16)
    h = _dot(y2, w1_ref[...]) + b1_ref[...].astype(f32)
    h = jax.nn.gelu(h, approximate=True).astype(jnp.bfloat16)
    mlp = _dot(h, w2_ref[...]) + b2_ref[...].astype(f32)

    o_ref[...] = (x + y + xn * dskip_ref[...].astype(f32) + mlp).astype(o_ref.dtype)


@jax.jit
def pallas_parallel_sum__ssm_conv_s4__mixer_channel_mlp__prompt_kernel(
    A_u: jax.Array,
    A_A_re: jax.Array,
    A_A_im: jax.Array,
    A_B_re: jax.Array,
    A_B_im: jax.Array,
    A_C_re: jax.Array,
    A_C_im: jax.Array,
    A_log_dt: jax.Array,
    A_Dskip: jax.Array,
    B_x: jax.Array,
    B_w1: jax.Array,
    B_b1: jax.Array,
    B_w2: jax.Array,
    B_b2: jax.Array,
):
    del B_x
    x = A_u.reshape(L, D)
    consts = [jnp.asarray(m) for m in _make_constants()]
    full = lambda a: pl.BlockSpec(a.shape, lambda c: (0,) * a.ndim)
    small = [A_A_re, A_A_im, A_B_re, A_B_im, A_C_re, A_C_im,
             A_log_dt.reshape(1, D), A_Dskip.reshape(1, D),
             B_w1, B_b1.reshape(1, FF), B_w2, B_b2.reshape(1, D)]
    args = [x] + small + consts
    in_specs = [pl.BlockSpec((B, D), lambda c: (c, 0))] + [full(a) for a in args[1:]]
    f32 = jnp.float32
    scratch = [
        pltpu.VMEM((NB, NF, D), f32),
        pltpu.VMEM((NB, NF, D), f32),
        pltpu.VMEM((NF, D), f32),
        pltpu.VMEM((FROWS, D), f32),
        pltpu.VMEM((7, N, D), f32),
        pltpu.VMEM((7, N, D), f32),
        pltpu.VMEM((4, N, 8, D), f32),
        pltpu.VMEM((4, N, 8, D), f32),
        pltpu.VMEM((16, N, D), f32),
        pltpu.VMEM((16, N, D), f32),
        pltpu.VMEM((N, D), f32),
        pltpu.VMEM((N, D), f32),
    ]
    out = pl.pallas_call(
        _kernel,
        grid=(NB,),
        in_specs=in_specs,
        out_specs=pl.BlockSpec((B, D), lambda c: (c, 0)),
        out_shape=jax.ShapeDtypeStruct((L, D), jnp.bfloat16),
        scratch_shapes=scratch,
        compiler_params=pltpu.CompilerParams(
            dimension_semantics=("arbitrary",),
            vmem_limit_bytes=110 * 1024 * 1024,
        ),
    )(*args)
    return out.reshape(1, L, D)
```

```python
import numpy as np
import jax
import jax.numpy as jnp
import jax.experimental.pallas as pl
import jax.experimental.pallas.tpu as pltpu

L, D, N, FF = 2048, 512, 128, 1792
B = 128
NB = L // B
NF = 2 * B
EPS = 1e-5

R = 16
NVALID = 641
FROWS = 768


def _row_lag(row):
    if row < 256:
        return row
    if row < 384:
        return 256 + 2 * (row - 256)
    if row < 512:
        return 512 + 4 * (row - 384)
    return 1024 + 8 * (row - 512)


def _block_row0(d):
    if d < 2:
        return d * B
    if d < 4:
        return 256 + (d - 2) * 64
    if d < 8:
        return 384 + (d - 4) * 32
    return 512 + (d - 8) * 16


def _split_bf16(a):
    hi = np.asarray(a, np.float64).astype(jnp.bfloat16)
    lo = (np.asarray(a, np.float64) - hi.astype(np.float64)).astype(jnp.bfloat16)
    return hi, lo


def _make_constants():
    k = np.arange(B)
    l = np.arange(B)
    theta = np.pi * (2 * k + 1) / (2 * B)
    ang = np.outer(theta, l)
    fwd = np.concatenate([np.cos(ang), -np.sin(ang)], 0)
    inv = np.concatenate([np.cos(ang.T), -np.sin(ang.T)], 1) / B
    lag_bf16 = np.arange(L).astype(jnp.bfloat16).astype(np.float64)
    frs = []
    for d in (0, 2, 4, 8):
        r0 = _block_row0(d)
        lags = np.array([_row_lag(r0 + j) if r0 + j < NVALID else -1.0 for j in range(B)], np.float64)
        rep = (lag_bf16[d * B:(d + 1) * B][:, None] == lags[None, :]).astype(np.float64)
        frs.append(fwd @ rep)
    km = np.stack(frs)
    consts = []
    for m in (fwd, inv, km):
        consts.extend(_split_bf16(m))
    return consts


def _layernorm(x):
    m = jnp.mean(x, axis=-1, keepdims=True)
    xc = x - m
    v = jnp.mean(xc * xc, axis=-1, keepdims=True)
    return xc * jax.lax.rsqrt(v + EPS)


def _dot(a, b):
    return jnp.dot(a, b, preferred_element_type=jnp.float32)


def _dot3(a_hi, a_lo, b):
    b_hi = b.astype(jnp.bfloat16)
    b_lo = (b - b_hi.astype(jnp.float32)).astype(jnp.bfloat16)
    return _dot(a_hi, b_hi) + (_dot(a_hi, b_lo) + _dot(a_lo, b_hi))


def _cmul(ar, ai, br, bi):
    return ar * br - ai * bi, ar * bi + ai * br


def _pairs_needed(c):
    return jnp.where(c < 2, 4 * (c + 1),
                     jnp.where(c < 4, 11 + 2 * (c - 2),
                               jnp.where(c < 8, 14 + (c - 4), 17 + (c - 7) // 2)))


def _kernel(x_ref, are_ref, aim_ref, bre_ref, bim_ref, cre_ref, cim_ref, logdt_ref, dskip_ref,
            w1_ref, b1_ref, w2_ref, b2_ref,
            fhi_ref, flo_ref, ihi_ref, ilo_ref, kmhi_ref, kmlo_ref,
            o_ref,
            uh_scr, kp_scr, khp_scr, f_scr, pw_re, pw_im, t_s, g_s, gc_re, gc_im):
    c = pl.program_id(0)
    f32 = jnp.float32

    @pl.when(c == 0)
    def _setup():
        dt = jnp.exp(logdt_ref[...].astype(f32)).astype(jnp.bfloat16).astype(f32)
        tr = lambda r: r[...].astype(f32).T
        a_r = tr(are_ref) * dt
        a_i = tr(aim_ref) * dt
        db_r = tr(bre_ref) * dt
        db_i = tr(bim_ref) * dt
        c_r = tr(cre_ref)
        c_i = tr(cim_ref)
        cb_r, cb_i = _cmul(c_r, c_i, db_r, db_i)
        gc_re[...] = cb_r
        gc_im[...] = cb_i
        for i in range(8):
            if i % 3 == 0:
                mag = jnp.exp(a_r * float(2 ** i))
                ph = a_i * float(2 ** i)
                er, ei = mag * jnp.cos(ph), mag * jnp.sin(ph)
            else:
                er, ei = er * er - ei * ei, 2.0 * er * ei
            pw_re[i] = er
            pw_im[i] = ei
        for t in range(D // 128):
            lanes = slice(t * 128, (t + 1) * 128)
            for j in range(4):
                tab = {}
                for r in range(1, R):
                    hb = r.bit_length() - 1
                    er, ei = pw_re[j + hb, :, lanes], pw_im[j + hb, :, lanes]
                    if r != (1 << hb):
                        er, ei = _cmul(er, ei, *tab[r - (1 << hb)])
                    tab[r] = (er, ei)
                    t_s[j, :, t, 2 * (r - 1)] = er.reshape(N // 8, 8, 128)
                    t_s[j, :, t, 2 * (r - 1) + 1] = ei.reshape(N // 8, 8, 128)
        khp_scr[...] = jnp.zeros_like(khp_scr)
        f_scr[...] = jnp.zeros_like(f_scr)

    x = x_ref[...].astype(f32)
    xn_b = _layernorm(x).astype(jnp.bfloat16)
    xn = xn_b.astype(f32)
    uh_scr[c] = _dot(fhi_ref[...], xn_b) + _dot(flo_ref[...], xn_b)

    sub = jax.lax.broadcasted_iota(jnp.int32, (8, 128), 0)

    def reduce8(accs):
        out = None
        for j, a_ in enumerate(accs):
            s_ = a_ + pltpu.roll(a_, 4, 0)
            s_ = s_ + pltpu.roll(s_, 2, 0)
            s_ = s_ + pltpu.roll(s_, 1, 0)
            out = s_ if out is None else jnp.where(sub == j, s_, out)
        return out

    def pair_body(p, carry):
        lv = jnp.where(p < 8, 0, jnp.where(p < 12, 1, jnp.where(p < 16, 2, 3)))
        sr_r = pw_re[4 + lv]
        sr_i = pw_im[4 + lv]
        g0r, g0i = gc_re[...], gc_im[...]
        g1r, g1i = _cmul(g0r, g0i, sr_r, sr_i)
        for t in range(D // 128):
            lanes = slice(t * 128, (t + 1) * 128)
            g_s[:, t, 0] = g0r[:, lanes].reshape(N // 8, 8, 128)
            g_s[:, t, 1] = g0i[:, lanes].reshape(N // 8, 8, 128)
            g_s[:, t, 2] = g1r[:, lanes].reshape(N // 8, 8, 128)
            g_s[:, t, 3] = g1i[:, lanes].reshape(N // 8, 8, 128)
        g2r, g2i = _cmul(g1r, g1i, sr_r, sr_i)
        gc_re[...] = g2r
        gc_im[...] = g2i

        def tile_body(t, carry2):
            lanes = pl.ds(pl.multiple_of(t * 128, 128), 128)
            for rg in range(R // 8):
                rs = list(range(rg * 8, rg * 8 + 8))

                def body(g, accs, rs=rs):
                    ts = [None if r == 0 else (t_s[lv, g, t, 2 * (r - 1)], t_s[lv, g, t, 2 * (r - 1) + 1])
                          for r in rs]
                    out = []
                    k = 0
                    for i in range(2):
                        gr_ = g_s[g, t, 2 * i]
                        gi_ = g_s[g, t, 2 * i + 1]
                        for tt in ts:
                            if tt is None:
                                out.append(accs[k] + gr_)
                            else:
                                out.append(accs[k] + (gr_ * tt[0] - gi_ * tt[1]))
                            k += 1
                    return tuple(out)
                accs = jax.lax.fori_loop(0, N // 8, body,
                                         tuple(jnp.zeros((8, 128), f32) for _ in range(16)),
                                         unroll=8)
                for i in range(2):
                    row = reduce8(accs[i * 8:(i + 1) * 8])
                    r_lo = p * (2 * R) + (i * R + rg * 8)
                    row = jnp.where(sub + r_lo < NVALID, row, 0.0)
                    f_scr[pl.ds(pl.multiple_of(r_lo, 8), 8), lanes] = row
            return carry2
        jax.lax.fori_loop(0, D // 128, tile_body, 0)
        return carry

    p_lo = jnp.where(c == 0, 0, _pairs_needed(c - 1))
    p_hi = _pairs_needed(c)
    jax.lax.fori_loop(p_lo, p_hi, pair_body, 0)

    kind = jnp.where(c < 2, 0, jnp.where(c < 4, 1, jnp.where(c < 8, 2, 3)))
    r0 = jnp.where(c < 2, c * B,
                   jnp.where(c < 4, 256 + (c - 2) * 64,
                             jnp.where(c < 8, 384 + (c - 4) * 32, 512 + (c - 8) * 16)))
    fb = f_scr[pl.ds(pl.multiple_of(r0, 16), B), :]
    kh = _dot3(kmhi_ref[kind], kmlo_ref[kind], fb)
    sgn = jnp.where((jax.lax.broadcasted_iota(jnp.int32, (B, D), 0) & 1) == 0, 1.0, -1.0)
    prev = khp_scr[...]
    kp_scr[c, :B, :] = kh[:B] - sgn * prev[B:]
    kp_scr[c, B:, :] = kh[B:] + sgn * prev[:B]
    khp_scr[...] = kh

    RC = 8
    zs = []
    for rc in range(B // RC):
        rows_r = pl.ds(rc * RC, RC)
        rows_i = pl.ds(B + rc * RC, RC)

        def term(dl, zr, zi, rows_r=rows_r, rows_i=rows_i):
            kr = kp_scr[dl, rows_r, :]
            ki = kp_scr[dl, rows_i, :]
            ur = uh_scr[c - dl, rows_r, :]
            ui = uh_scr[c - dl, rows_i, :]
            return zr + (kr * ur - ki * ui), zi + (kr * ui + ki * ur)

        def zbody(k, carry):
            zr, zi = term(2 * k + 1, *carry)
            return term(2 * k + 2, zr, zi)
        zr, zi = term(0, jnp.zeros((RC, D), f32), jnp.zeros((RC, D), f32))
        zr, zi = jax.lax.fori_loop(0, c // 2, zbody, (zr, zi))
        zr, zi = jax.lax.cond(c % 2 == 1, lambda a_, b_: term(c, a_, b_), lambda a_, b_: (a_, b_), zr, zi)
        zs.append((zr, zi))
    z = jnp.concatenate([zz[0] for zz in zs] + [zz[1] for zz in zs], axis=0)
    y = _dot3(ihi_ref[...], ilo_ref[...], z)

    y2 = _layernorm(xn).astype(jnp.bfloat16)
    h = _dot(y2, w1_ref[...]) + b1_ref[...].astype(f32)
    h = jax.nn.gelu(h, approximate=True).astype(jnp.bfloat16)
    mlp = _dot(h, w2_ref[...]) + b2_ref[...].astype(f32)

    o_ref[...] = (x + y + xn * dskip_ref[...].astype(f32) + mlp).astype(o_ref.dtype)


@jax.jit
def pallas_parallel_sum__ssm_conv_s4__mixer_channel_mlp__prompt_kernel(
    A_u: jax.Array,
    A_A_re: jax.Array,
    A_A_im: jax.Array,
    A_B_re: jax.Array,
    A_B_im: jax.Array,
    A_C_re: jax.Array,
    A_C_im: jax.Array,
    A_log_dt: jax.Array,
    A_Dskip: jax.Array,
    B_x: jax.Array,
    B_w1: jax.Array,
    B_b1: jax.Array,
    B_w2: jax.Array,
    B_b2: jax.Array,
):
    del B_x
    x = A_u.reshape(L, D)
    consts = [jnp.asarray(m) for m in _make_constants()]
    full = lambda a: pl.BlockSpec(a.shape, lambda c: (0,) * a.ndim)
    small = [A_A_re, A_A_im, A_B_re, A_B_im, A_C_re, A_C_im,
             A_log_dt.reshape(1, D), A_Dskip.reshape(1, D),
             B_w1, B_b1.reshape(1, FF), B_w2, B_b2.reshape(1, D)]
    args = [x] + small + consts
    in_specs = [pl.BlockSpec((B, D), lambda c: (c, 0))] + [full(a) for a in args[1:]]
    f32 = jnp.float32
    scratch = [
        pltpu.VMEM((NB, NF, D), f32),
        pltpu.VMEM((NB, NF, D), f32),
        pltpu.VMEM((NF, D), f32),
        pltpu.VMEM((FROWS, D), f32),
        pltpu.VMEM((8, N, D), f32),
        pltpu.VMEM((8, N, D), f32),
        pltpu.VMEM((4, N // 8, D // 128, 2 * (R - 1), 8, 128), f32),
        pltpu.VMEM((N // 8, D // 128, 4, 8, 128), f32),
        pltpu.VMEM((N, D), f32),
        pltpu.VMEM((N, D), f32),
    ]
    out = pl.pallas_call(
        _kernel,
        grid=(NB,),
        in_specs=in_specs,
        out_specs=pl.BlockSpec((B, D), lambda c: (c, 0)),
        out_shape=jax.ShapeDtypeStruct((L, D), jnp.bfloat16),
        scratch_shapes=scratch,
        compiler_params=pltpu.CompilerParams(
            dimension_semantics=("arbitrary",),
            vmem_limit_bytes=110 * 1024 * 1024,
        ),
    )(*args)
    return out.reshape(1, L, D)
```
